```python
import jax
import jax.numpy as jnp

def _softmax(x, axis=-1):
    return jax.nn.softmax(x, axis=axis)
def _gelu(x):
    return jax.nn.gelu(x, approximate=True)
def _silu(x):
    return jax.nn.silu(x)
def _sigmoid(x):
    return jax.nn.sigmoid(x)
def _layernorm(x, axis=-1, eps=1e-5):
    m = jnp.mean(x, axis=axis, keepdims=True)
    v = jnp.var(x, axis=axis, keepdims=True)
    return (x - m) / jnp.sqrt(v + eps)
def _scatter_add(tgt, idx, src, axis=0):
    return tgt.at[idx].add(src)
def _segment_sum(src, seg, n):
    return jax.ops.segment_sum(src, seg, n)
class _Rng:
    def __init__(self, key):
        self._k = key
    def _next(self):
        self._k, sub = jax.random.split(self._k)
        return sub
    def normal(self, shape):
        return jax.random.normal(self._next(), shape, dtype=jnp.bfloat16)
    def randint(self, lo, hi, shape):
        return jax.random.randint(self._next(), shape, lo, hi, dtype=jnp.int32)
    def uniform(self, shape, lo=0.0, hi=1.0):
        return jax.random.uniform(self._next(), shape, jnp.bfloat16, lo, hi)
    def permutation(self, n):
        return jax.random.permutation(self._next(), n)


kernel_name = 'standalone__fused_io_aware_attn__prompt'

def setup_inputs():
    _rng = _Rng(jax.random.key(int.from_bytes(__import__("os").urandom(4), "little")))
    _w = (lambda a: (lambda t: t.astype(jnp.bfloat16) if jnp.issubdtype(t.dtype, jnp.floating) else t)(jnp.asarray(a)))
    B, H, S = 2, 32, 2048
    Dh = max(1, 1024 // 32)
    return {
        "q": _w((lambda *s: _rng.normal(s) * 0.05)(B, H, S, Dh)),
        "k": _w((lambda *s: _rng.normal(s) * 0.05)(B, H, S, Dh)),
        "v": _w((lambda *s: _rng.normal(s) * 0.05)(B, H, S, Dh)),
    }

def reference(q, k, v):
    scale = q.shape[-1] ** -0.5
    s = jnp.einsum('bhqd,bhkd->bhqk', q, k) * scale
    p = _softmax(s, axis=-1)
    return jnp.einsum('bhqk,bhkd->bhqd', p, v)
```

```python
import functools

import jax
import jax.numpy as jnp
from jax import lax
import jax.experimental.pallas as pl
import jax.experimental.pallas.tpu as pltpu

LOG2E = 1.4426950408889634
L_LO, L_HI = 2.0 ** -24, 2.0 ** 40
BK, QB, G, PVLEAD = 128, 512, 2, 2
F32, BF16 = jnp.float32, jnp.bfloat16


def _kernel(q_hbm, k_hbm, v_hbm, o_hbm, q_all, k_all, v_all, o_all,
            k_scr, p_scr, l_scr, lprev_scr, acc_scr, bad_scr, sems):
    N, D, S = q_all.shape
    NG, NK, NQ = N // G, S // BK, S // QB
    scale = D ** -0.5

    def cp(j, g):
        sl = pl.ds(g * G, G)
        src, dst = ((q_hbm, q_all), (k_hbm, k_all), (v_hbm, v_all), (o_all, o_hbm))[j]
        return pltpu.make_async_copy(src.at[sl], dst.at[sl], sems.at[j, g])

    def xpose(kt):
        return jnp.concatenate([kt] * (128 // D), axis=0).T

    def body(do_qk, do_pv, h):
        if do_qk:
            hn = jnp.minimum(h + 1, N - 1) if do_pv else h + 1
            qf = q_all[h].astype(F32) * (scale * LOG2E)
            hi = qf.astype(BF16)
            lo = (qf - hi.astype(F32)).astype(BF16)
            qw = jnp.concatenate([hi, lo], axis=0)
        if do_pv:
            lprev_scr[...] = l_scr[...]
        bad = []

        def pv(u):
            kc, q0 = u // NQ, (u % NQ) * QB
            q1, k0, k1 = q0 + QB, kc * BK, (kc + 1) * BK
            pb = pltpu.bitcast(p_scr[k0 // 2:k1 // 2, q0:q1], BF16)
            o = jnp.dot(v_all[h - 1, :, k0:k1], pb, preferred_element_type=F32)
            if kc == 0:
                acc_scr[:, q0:q1] = o
            elif kc < NK - 1:
                acc_scr[:, q0:q1] += o
            else:
                l = jnp.sum(lprev_scr[:, q0:q1], axis=0, keepdims=True)
                res = (acc_scr[:, q0:q1] + o) * (1.0 / l)
                o_all[h - 1, :, q0:q1] = res.astype(o_all.dtype)
                nonfinite = jnp.where(jnp.abs(res) < jnp.inf, 0.0, 1.0)
                nonfinite = jnp.max(nonfinite.reshape(D // 8, 8, QB), axis=0)
                okl = jnp.logical_and(l >= L_LO, l <= L_HI)
                bad.append(jnp.maximum(nonfinite, jnp.where(okl, 0.0, 1.0)))

        def qk(u):
            kc, q0 = u // NQ, (u % NQ) * QB
            q1, k0, k1 = q0 + QB, kc * BK, (kc + 1) * BK
            st = jnp.dot(k_scr[k0:k1, 0:2 * D], qw[:, q0:q1], preferred_element_type=F32)
            p = jnp.exp2(st)
            ls = jnp.sum(p.reshape(BK // 8, 8, QB), axis=0)
            l_scr[:, q0:q1] = ls if kc == 0 else l_scr[:, q0:q1] + ls
            p_scr[k0 // 2:k1 // 2, q0:q1] = pltpu.bitcast(p.astype(BF16), jnp.uint32)
            if u % NQ == NQ - 1:
                k_scr[k0:k1, :] = xpose(k_all[hn, :, k0:k1])

        pvi = 0
        for u in range(NK * NQ):
            while do_pv and pvi < min(NK * NQ, u + PVLEAD):
                pv(pvi)
                pvi += 1
            if do_qk:
                qk(u)
        if do_pv:
            bv = functools.reduce(jnp.maximum, bad)
            bad_scr[h - 1] = functools.reduce(
                jnp.maximum, [bv[:, i:i + 128] for i in range(0, QB, 128)])

    def safe_head(h):
        def qb(i, carry):
            q0 = pl.multiple_of(i * QB, QB)
            qt = q_all[h, :, pl.ds(q0, QB)]

            def kb(j, cr):
                m, l, acc = cr
                k0 = pl.multiple_of(j * BK, BK)
                k = xpose(k_all[h, :, pl.ds(k0, BK)])[:, 0:D]
                st = jnp.dot(k, qt, preferred_element_type=F32) * scale
                mn = jnp.maximum(m, jnp.max(st, axis=0, keepdims=True))
                al = jnp.exp(m - mn)
                p = jnp.exp(st - mn)
                l = al * l + jnp.sum(p, axis=0, keepdims=True)
                acc = al * acc + jnp.dot(v_all[h, :, pl.ds(k0, BK)], p.astype(BF16),
                                         preferred_element_type=F32)
                return mn, l, acc

            init = (jnp.full((1, QB), -jnp.inf, F32), jnp.zeros((1, QB), F32),
                    jnp.zeros((D, QB), F32))
            m, l, acc = lax.fori_loop(0, NK, kb, init)
            o_all[h, :, pl.ds(q0, QB)] = (acc / l).astype(o_all.dtype)
            return carry

        lax.fori_loop(0, NQ, qb, 0)

    for j in (1, 0, 2):
        cp(j, 0).start()
    cp(1, 0).wait()
    cp(0, 0).wait()
    for j in (1, 0, 2):
        cp(j, 1).start()
    for kc in range(NK):
        k_scr[kc * BK:(kc + 1) * BK, :] = xpose(k_all[0, :, kc * BK:(kc + 1) * BK])
    body(True, False, 0)
    cp(2, 0).wait()

    def step(h, carry):
        @pl.when(h % G == G - 1)
        def _():
            g = h // G

            @pl.when(g + 1 < NG)
            def _():
                for j in (1, 0, 2):
                    cp(j, g + 1).wait()

            @pl.when(g + 2 < NG)
            def _():
                for j in (1, 0, 2):
                    cp(j, g + 2).start()

            @pl.when(g > 0)
            def _():
                cp(3, g - 1).start()

        body(True, True, h)
        return carry

    lax.fori_loop(1, N, step, 0)
    body(False, True, N)
    cp(3, NG - 1).start()
    for g in range(NG):
        cp(3, g).wait()

    @pl.when(jnp.max(jnp.max(bad_scr[...], axis=0)) > 0.0)
    def _():
        def redo(h, carry):
            @pl.when(jnp.max(bad_scr[h]) > 0.0)
            def _():
                safe_head(h)
                d = pltpu.make_async_copy(o_all.at[h], o_hbm.at[h], sems.at[3, 0])
                d.start()
                d.wait()
            return carry

        lax.fori_loop(0, N, redo, 0)


@jax.jit
def pallas_standalone__fused_io_aware_attn__prompt_kernel(q, k, v):
    B, H, S, D = q.shape
    N = B * H
    qt, kt, vt = (jnp.swapaxes(x, 2, 3).reshape(N, D, S) for x in (q, k, v))
    anyspec = pl.BlockSpec(memory_space=pl.ANY)
    ot = pl.pallas_call(
        _kernel,
        in_specs=[anyspec] * 3,
        out_specs=anyspec,
        out_shape=jax.ShapeDtypeStruct((N, D, S), q.dtype),
        scratch_shapes=[pltpu.VMEM((N, D, S), BF16)] * 4 + [
            pltpu.VMEM((S, 128), BF16),
            pltpu.VMEM((S // 2, S), jnp.uint32),
            pltpu.VMEM((8, S), F32),
            pltpu.VMEM((8, S), F32),
            pltpu.VMEM((D, S), F32),
            pltpu.VMEM((N, 8, 128), F32),
            pltpu.SemaphoreType.DMA((4, N // G)),
        ],
        compiler_params=pltpu.CompilerParams(vmem_limit_bytes=64 * 2**20),
    )(qt, kt, vt)
    return jnp.swapaxes(ot.reshape(B, H, D, S), 2, 3)
```
